```python
import os as _os
_os.environ.setdefault("JAX_PLATFORMS", "cpu")
import jax
import jax.numpy as jnp

def _softmax(x, axis=-1):
    return jax.nn.softmax(x, axis=axis)
def _gelu(x):
    return jax.nn.gelu(x, approximate=True)
def _silu(x):
    return jax.nn.silu(x)
def _sigmoid(x):
    return jax.nn.sigmoid(x)
def _layernorm(x, axis=-1, eps=1e-5):
    m = jnp.mean(x, axis=axis, keepdims=True)
    v = jnp.var(x, axis=axis, keepdims=True)
    return (x - m) / jnp.sqrt(v + eps)
def _scatter_add(tgt, idx, src, axis=0):
    return tgt.at[idx].add(src)
def _segment_sum(src, seg, n):
    return jax.ops.segment_sum(src, seg, n)
class _Rng:
    def __init__(self, key):
        self._k = key
    def _next(self):
        self._k, sub = jax.random.split(self._k)
        return sub
    def normal(self, shape):
        return jax.random.normal(self._next(), shape, dtype=jnp.bfloat16)
    def randint(self, lo, hi, shape):
        return jax.random.randint(self._next(), shape, lo, hi, dtype=jnp.int32)
    def uniform(self, shape, lo=0.0, hi=1.0):
        return jax.random.uniform(self._next(), shape, jnp.bfloat16, lo, hi)
    def permutation(self, n):
        return jax.random.permutation(self._next(), n)


kernel_name = 'sequential_preLN__mha_block__moe_arch_mod__prompt'

def setup_inputs():
    _rng = _Rng(jax.random.key(int.from_bytes(__import__("os").urandom(4), "little")))
    _w = (lambda a: (lambda t: t.astype(jnp.bfloat16) if jnp.issubdtype(t.dtype, jnp.floating) else t)(jnp.asarray(a)))
    def _A_setup():
        B, S, D, H = 1, 2048, 512, 32
        return {
            "x": _w((lambda *s: _rng.normal(s) * 0.05)(B, S, D)),
            "wqkv": _w((lambda *s: _rng.normal(s) * 0.05)(D, 3 * D)),
            "wo": _w((lambda *s: _rng.normal(s) * 0.05)(D, D)),
        }
    _A_in = _A_setup()

    def _B_setup():
        B, S, D, F, C = 1, 2048, 512, 1792, 2
        return {
            "x": _w((lambda *s: _rng.normal(s) * 0.05)(B, S, D)),
            "w_r": _w((lambda *s: _rng.normal(s) * 0.05)(D)),
            "w_gate": _w((lambda *s: _rng.normal(s) * 0.05)(D, F)),
            "w_up": _w((lambda *s: _rng.normal(s) * 0.05)(D, F)),
            "w_down": _w((lambda *s: _rng.normal(s) * 0.05)(F, D)),
        }
    _B_in = _B_setup()

    return {
        "A_x": _A_in["x"],
        "A_wqkv": _A_in["wqkv"],
        "A_wo": _A_in["wo"],
        "B_x": _B_in["x"],
        "B_w_r": _B_in["w_r"],
        "B_w_gate": _B_in["w_gate"],
        "B_w_up": _B_in["w_up"],
        "B_w_down": _B_in["w_down"],
    }

def reference(A_x, A_wqkv, A_wo, B_x, B_w_r, B_w_gate, B_w_up, B_w_down):
    def _A_ref(x, wqkv, wo):
        B, S, D = x.shape
        H = 32
        Dh = D // H
        qkv = (lambda x, *d: x.transpose(*d))((x @ wqkv).reshape(B, S, 3, H, Dh), 2, 0, 3, 1, 4)
        q, k, v = qkv[0], qkv[1], qkv[2]
        scores = jnp.einsum("bhqd,bhkd->bhqk", q, k) * (Dh ** -0.5)
        p = _softmax(scores, axis=-1)
        o = jnp.einsum("bhqk,bhkd->bhqd", p, v)
        return (lambda x, *d: x.transpose(*d))(o, 0, 2, 1, 3).reshape(B, S, D) @ wo

    def _B_ref(x, w_r, w_gate, w_up, w_down):
        B, S, D = x.shape
        C = 2
        r = x @ w_r
        idx = jnp.argsort(-r, axis=-1)[:, :C]
        idx_e = jnp.repeat(idx.reshape(B, C, 1), D, axis=2)
        x_sel = jnp.take_along_axis(x, idx_e, axis=1)
        g = _silu(x_sel @ w_gate)
        u = x_sel @ w_up
        y = (g * u) @ w_down
        r_sel = _sigmoid(jnp.take_along_axis(r, idx, axis=1))
        y = y * r_sel.reshape(B, C, 1)
        b_off = (jnp.arange(B) * S).reshape(B, 1)
        flat_idx = (idx + b_off).reshape(B * C)
        zero = (x * 0.0).reshape(B * S, D)
        upd = _scatter_add(zero, flat_idx, y.reshape(B * C, D), axis=0)
        return x + upd.reshape(B, S, D)

    x = A_x
    h = x + _A_ref(_layernorm(x, axis=-1), A_wqkv, A_wo)
    h2 = h + _B_ref(_layernorm(h, axis=-1), B_w_r, B_w_gate, B_w_up, B_w_down)
    return h2
```

```python
import math

import jax
import jax.numpy as jnp
from jax import lax
import jax.experimental.pallas as pl
import jax.experimental.pallas.tpu as pltpu

f32 = jnp.float32
bf16 = jnp.bfloat16
u32 = jnp.uint32
i32 = jnp.int32

S = 2048
D = 512
H = 32
DH = 16
F = 1792
EPS = 1e-5

TM = 256
TQ = 512
KC = 128
NQ = S // TQ
NC = S // KC
T = H * NQ
NSUB = NQ
LAG = 2
DEL = 2
NZ = NSUB * NC
ORDER = (14, 15, 12, 13, 10, 11, 8, 9, 6, 7, 4, 5, 2, 3, 0, 1)
QSCALE = (DH ** -0.5) * math.log2(math.e)
NT = (((1,), (1,)), ((), ()))


def _ln(xf):
    m = jnp.mean(xf, axis=-1, keepdims=True)
    xc = xf - m
    v = jnp.mean(xc * xc, axis=-1, keepdims=True)
    return xc * lax.rsqrt(v + EPS)


def _to_u32(x):
    return pltpu.bitcast(x.astype(bf16), u32)


def _kernel(x_ref, wqkv_ref, wo_ref, wr_ref, wg_hbm, wu_hbm, wd_hbm, o_ref,
            wg_s, wu_s, wd_s, wsem,
            wqvt_s, k_s, qt_s, vt_s, ot_s, w_s, z_s, s_scr, xn2_s, r_s):
    cp_g = pltpu.make_async_copy(wg_hbm, wg_s, wsem.at[0])
    cp_u = pltpu.make_async_copy(wu_hbm, wu_s, wsem.at[1])
    cp_d = pltpu.make_async_copy(wd_hbm, wd_s, wsem.at[2])
    cp_g.start()
    cp_u.start()
    cp_d.start()

    for i in range(NZ):
        z_s[i] = 0

    ri = lax.broadcasted_iota(i32, (128, 128), 0)
    ci = lax.broadcasted_iota(i32, (128, 128), 1)
    eye = jnp.where(ri == ci, 1.0, 0.0).astype(bf16)

    for b in range(4):
        wq = wqkv_ref[:, b * 128:(b + 1) * 128]
        wv = wqkv_ref[:, 2 * D + b * 128:2 * D + (b + 1) * 128]
        wqvt_s[b * 64:(b + 1) * 64, :] = _to_u32(
            lax.dot_general(eye, wq, NT, preferred_element_type=f32))
        wqvt_s[256 + b * 64:256 + (b + 1) * 64, :] = _to_u32(
            lax.dot_general(eye, wv, NT, preferred_element_type=f32))

    def proj(i, carry):
        r0 = pl.multiple_of(i * TM, TM)
        xn = _ln(x_ref[pl.ds(r0, TM), :].astype(f32)).astype(bf16)
        k = jnp.dot(xn, wqkv_ref[:, D:2 * D], preferred_element_type=f32)
        k_s[pl.ds(pl.multiple_of(i * (TM // 2), TM // 2), TM // 2), :] = _to_u32(k)
        qv = lax.dot_general(pltpu.bitcast(wqvt_s[...], bf16), xn, NT,
                             preferred_element_type=f32)
        qt_s[:, pl.ds(r0, TM)] = _to_u32(qv[:D] * QSCALE)
        vt_s[:, pl.ds(r0, TM)] = _to_u32(qv[D:])
        return carry

    lax.fori_loop(0, S // TM, proj, 0)

    def w_val(t):
        h = t // NQ
        qi = t % NQ
        qh = qt_s[pl.ds(pl.multiple_of(h * 8, 8), 8),
                  pl.ds(pl.multiple_of(qi * TQ, TQ), TQ)]
        rows = lax.broadcasted_iota(i32, (64, TQ), 0) // 8
        return jnp.where(rows == h % 8, jnp.tile(qh, (8, 1)), jnp.zeros((), u32))

    def qk(c, t, w, slot, m_run):
        goff = pl.multiple_of(((t // NQ) // 8) * 128, 128)
        kk = pltpu.bitcast(k_s[c * KC // 2:(c + 1) * KC // 2, pl.ds(goff, 128)], bf16)
        s = jnp.dot(kk, pltpu.bitcast(w, bf16), preferred_element_type=f32)
        s_scr[slot, c * KC:(c + 1) * KC, :] = s
        for i in range(KC // 8):
            x = s[8 * i:8 * i + 8]
            m_run = x if m_run is None else jnp.maximum(m_run, x)
        return m_run

    def sm(c, t, slot, m, l, acc):
        so = s_scr[slot, c * KC:(c + 1) * KC, :]
        p = jnp.exp2(so.reshape(KC // 8, 8, TQ) - m[None])
        for i in ORDER:
            l = p[i] if l is None else l + p[i]
        hoff = pl.multiple_of((t // NQ) * 8, 8)
        vt = pltpu.bitcast(vt_s[pl.ds(hoff, 8), c * KC:(c + 1) * KC], bf16)
        a = jnp.dot(vt, p.reshape(KC, TQ).astype(bf16), preferred_element_type=f32)
        return l, (a if acc is None else acc + a)

    def fin(t, l, acc):
        hoff = pl.multiple_of((t // NQ) * 8, 8)
        lt = jnp.sum(l, axis=0, keepdims=True)
        ot_s[pl.ds(hoff, 8), pl.ds(pl.multiple_of((t % NQ) * TQ, TQ), TQ)] = _to_u32(
            acc * pl.reciprocal(lt, approx=False))

    def colmax(mr):
        return jnp.broadcast_to(jnp.max(mr, axis=0, keepdims=True), (8, TQ))

    w0 = w_val(0)
    mr0 = None
    for c in range(NC):
        mr0 = qk(c, 0, w0, 0, mr0)
    m_cur0 = colmax(mr0)
    s_scr[1, (NC - LAG) * KC:, :] = jnp.zeros((LAG * KC, TQ), f32)
    w_s[0] = w_val(1)

    def attn(it, carry):
        m_prev, m_cur, l, acc = carry
        hist = []
        n = 0
        for u in range(NSUB):
            t = it * NSUB + u
            tn = jnp.minimum(t + 1, T - 1)
            tp = jnp.maximum(t - 1, 0)
            sc = u % 2
            sn = 1 - sc
            mr = None
            for c in range(NC):
                w = w_s[u % 2 + z_s[n]]
                n += 1
                mr = qk(c, tn, w, sn, mr)
                hist.append(mr)
                if len(hist) > DEL:
                    dep = hist[-1 - DEL]
                    tie = lambda m, dep=dep: jnp.minimum(m, jnp.maximum(m, dep))
                else:
                    tie = lambda m: m
                if c < LAG:
                    l, acc = sm(NC - LAG + c, tp, sn, tie(m_prev), l, acc)
                    if c == LAG - 1:
                        fin(tp, l, acc)
                        l = None
                        acc = None
                else:
                    l, acc = sm(c - LAG, t, sc, tie(m_cur), l, acc)
                if c == 8:
                    w_s[1 - u % 2] = w_val(jnp.minimum(t + 2, T - 1))
            m_prev = m_cur
            m_cur = colmax(mr)
        return m_prev, m_cur, l, acc

    init = (jnp.zeros((8, TQ), f32), m_cur0, jnp.ones((8, TQ), f32),
            jnp.zeros((DH, TQ), f32))
    m_prev, _, l, acc = lax.fori_loop(0, T // NSUB, attn, init)
    for c in range(LAG):
        l, acc = sm(NC - LAG + c, T - 1, (T - 1) % 2, m_prev, l, acc)
    fin(T - 1, l, acc)

    wr = wr_ref[...].astype(f32)

    def outp(i, carry):
        r0 = pl.multiple_of(i * TM, TM)
        rows = []
        for b in range(TM // 128):
            ot = pltpu.bitcast(
                ot_s[:, pl.ds(pl.multiple_of(r0 + b * 128, 128), 128)], bf16)
            rows.append(lax.dot_general(eye, ot, NT, preferred_element_type=f32))
        o = jnp.concatenate(rows, axis=0).astype(bf16)
        attn_out = jnp.dot(o, wo_ref[...], preferred_element_type=f32)
        h = (x_ref[pl.ds(r0, TM), :].astype(f32) + attn_out).astype(bf16).astype(f32)
        xn2 = _ln(h).astype(bf16)
        xn2_s[pl.ds(r0, TM), :] = xn2
        xn2f = xn2.astype(f32)
        r = jnp.sum(xn2f * wr, axis=-1, keepdims=True)
        r_s[pl.ds(r0, TM), :] = r.astype(bf16).astype(f32)
        o_ref[pl.ds(r0, TM), :] = (h + xn2f).astype(bf16)
        return carry

    lax.fori_loop(0, S // TM, outp, 0)

    r = r_s[...]
    idx = lax.broadcasted_iota(i32, (S, 1), 0)
    r1 = jnp.max(r)
    i1 = jnp.min(jnp.where(r == r1, idx, S))
    rm = jnp.where(idx == i1, -jnp.inf, r)
    r2 = jnp.max(rm)
    i2 = jnp.min(jnp.where((rm == r2) & (idx != i1), idx, S))
    i1 = jnp.minimum(i1, S - 1)
    i2 = jnp.minimum(i2, S - 1)

    row16 = lax.broadcasted_iota(i32, (16, D), 0)
    b1 = pl.multiple_of((i1 // 16) * 16, 16)
    b2 = pl.multiple_of((i2 // 16) * 16, 16)
    blk1 = xn2_s[pl.ds(b1, 16), :].astype(f32)
    blk2 = xn2_s[pl.ds(b2, 16), :].astype(f32)
    x1 = jnp.sum(jnp.where(row16 == i1 % 16, blk1, 0.0), axis=0, keepdims=True)
    x2 = jnp.sum(jnp.where(row16 == i2 % 16, blk2, 0.0), axis=0, keepdims=True)
    xs = jnp.where(row16 == 0, x1, jnp.where(row16 == 1, x2, 0.0)).astype(bf16)

    cp_g.wait()
    cp_u.wait()
    cp_d.wait()
    g = jnp.dot(xs, wg_s[...], preferred_element_type=f32)
    g = g * jax.nn.sigmoid(g)
    uu = jnp.dot(xs, wu_s[...], preferred_element_type=f32)
    y = jnp.dot((g * uu).astype(bf16), wd_s[...], preferred_element_type=f32)
    gate = jax.nn.sigmoid(jnp.where(row16 == 0, r1, r2))
    y = y * gate
    y1 = y[0:1]
    y2 = y[1:2]

    ob = o_ref[pl.ds(b1, 16), :].astype(f32)
    o_ref[pl.ds(b1, 16), :] = jnp.where(row16 == i1 % 16, ob + y1, ob).astype(bf16)
    ob = o_ref[pl.ds(b2, 16), :].astype(f32)
    o_ref[pl.ds(b2, 16), :] = jnp.where(row16 == i2 % 16, ob + y2, ob).astype(bf16)


@jax.jit
def pallas_sequential_preLN__mha_block__moe_arch_mod__prompt_kernel(
    A_x: jax.Array,
    A_wqkv: jax.Array,
    A_wo: jax.Array,
    B_x: jax.Array,
    B_w_r: jax.Array,
    B_w_gate: jax.Array,
    B_w_up: jax.Array,
    B_w_down: jax.Array,
):
    del B_x
    vm = pl.BlockSpec(memory_space=pltpu.VMEM)
    hbm = pl.BlockSpec(memory_space=pl.ANY)
    out = pl.pallas_call(
        _kernel,
        out_shape=jax.ShapeDtypeStruct((S, D), bf16),
        in_specs=[vm, vm, vm, vm, hbm, hbm, hbm],
        out_specs=vm,
        scratch_shapes=[
            pltpu.VMEM((D, F), bf16),
            pltpu.VMEM((D, F), bf16),
            pltpu.VMEM((F, D), bf16),
            pltpu.SemaphoreType.DMA((3,)),
            pltpu.VMEM((D, D), u32),
            pltpu.VMEM((S // 2, D), u32),
            pltpu.VMEM((D // 2, S), u32),
            pltpu.VMEM((D // 2, S), u32),
            pltpu.VMEM((D // 2, S), u32),
            pltpu.VMEM((2, 64, TQ), u32),
            pltpu.SMEM((NZ,), i32),
            pltpu.VMEM((2, S, TQ), f32),
            pltpu.VMEM((S, D), bf16),
            pltpu.VMEM((S, 1), f32),
        ],
        compiler_params=pltpu.CompilerParams(vmem_limit_bytes=100 * 1024 * 1024),
        name="preln_mha_mod",
    )(A_x.reshape(S, D), A_wqkv, A_wo, B_w_r.reshape(1, D),
      B_w_gate, B_w_up, B_w_down)
    return out.reshape(1, S, D)
```

```python
import functools
import math

import jax
import jax.numpy as jnp
from jax import lax
import jax.experimental.pallas as pl
import jax.experimental.pallas.tpu as pltpu

f32 = jnp.float32
bf16 = jnp.bfloat16
u32 = jnp.uint32
i32 = jnp.int32

S = 2048
D = 512
H = 32
DH = 16
F = 1792
EPS = 1e-5

TM = 256
NTILE = S // TM
TQ = 512
KC = 128
NQ = S // TQ
NC = S // KC
HB = 2
NSUB = NQ * HB
NZ = NSUB * NC
RV = 16
NB = (KC - RV) // 16
VB = 6
SLOT = tuple(i for i in range(8) if i != VB) + (VB,)
RING = 4
PL = 3
OFF = 4
AK = 2
AB = RING * KC
MR = AB + 32
QSCALE = (DH ** -0.5) * math.log2(math.e)
NT = (((1,), (1,)), ((), ()))
TN = (((0,), (0,)), ((), ()))
L_MAX = 2.0 ** 100
L_MIN = 2.0 ** -40
V_MAX = 2.0 ** 24

G0 = PL
GE = 58
GSCHED = {}
for _m in range(NC * DH):
    GSCHED.setdefault(G0 + (_m * (GE - G0)) // (NC * DH), {}).setdefault(
        _m // DH, []).append(_m % DH)


def _ln(xf):
    m = jnp.mean(xf, axis=-1, keepdims=True)
    xc = xf - m
    v = jnp.mean(xc * xc, axis=-1, keepdims=True)
    return xc * lax.rsqrt(v + EPS)


def _to_u32(x):
    return pltpu.bitcast(x.astype(bf16), u32)


def _kernel(x_hbm, wqkv_hbm, wo_hbm, wr_hbm, wg_hbm, wu_hbm, wd_hbm, o_hbm,
            x_ref, wqkv_ref, wo_ref, wr_ref, wg_s, wu_s, wd_s, o_ref,
            xsem, wsem, osem,
            wqvt_s, k_s, mem, qt_s, vt_s, ot_s, qb_s, kb0, kb1, z_s,
            l_s, xn2_s, r_s):
    kb_s = (kb0, kb1)
    xcut = (0, TM, 2 * TM, S)
    cp_x = [pltpu.make_async_copy(x_hbm.at[xcut[i]:xcut[i + 1]], x_ref.at[xcut[i]:xcut[i + 1]],
                                  xsem.at[i]) for i in range(3)]
    wcut = ((0, 256), (2 * D, 2 * D + 256), (256, D), (2 * D + 256, 3 * D), (D, 2 * D))
    cp_w = [pltpu.make_async_copy(wqkv_hbm.at[:, a:b], wqkv_ref.at[:, a:b], wsem.at[8 + p])
            for p, (a, b) in enumerate(wcut)]
    cp_o = pltpu.make_async_copy(wo_hbm, wo_ref, wsem.at[3])
    cp_r = pltpu.make_async_copy(wr_hbm, wr_ref, wsem.at[4])
    cp_g = pltpu.make_async_copy(wg_hbm, wg_s, wsem.at[5])
    cp_u = pltpu.make_async_copy(wu_hbm, wu_s, wsem.at[6])
    cp_d = pltpu.make_async_copy(wd_hbm, wd_s, wsem.at[7])
    cp_x[0].start()
    cp_w[0].start()
    cp_w[1].start()

    for i in range(NZ + 8):
        z_s[i] = 0
    mem[(RING - PL) * KC:, :] = jnp.zeros((MR - (RING - PL) * KC, D), u32)
    kb1[0, NC - PL + 1:] = jnp.zeros((PL - 1, DH, RV, 128), f32)

    def transpose_w(g):
        for col0, row0 in ((0, 0), (2 * D, 8)):
            wt = pltpu.bitcast(wqkv_ref[:, col0 + g * 128:col0 + (g + 1) * 128].T, u32)
            for j in range(8):
                r = (g * 8 + j) * 16 + row0
                wqvt_s[r:r + 8, :] = wt[8 * j:8 * j + 8]

    kref = [None] * 4
    vmax = [None]

    def proj_k(i, g, xn):
        k = jnp.dot(xn, wqkv_ref[:, D + g * 128:D + (g + 1) * 128],
                    preferred_element_type=f32)
        if kref[g] is None:
            kref[g] = jnp.mean(k, axis=0, keepdims=True)
        k = k - kref[g]
        for cc in range(TM // KC):
            c = i * (TM // KC) + cc
            kc = k[cc * KC:(cc + 1) * KC]
            xm = _to_u32(jnp.concatenate([kc[16 * p:16 * p + 16] for p in SLOT], axis=0))
            for j in range(8):
                a = pltpu.roll(xm, 128 - 16 * j, 1) if j else xm
                row = (g * 8 + j) * NC * 16 + c * 16
                for n_ in range(8):
                    k_s[row + (n_ // 4) * 8:row + (n_ // 4) * 8 + 8,
                        (n_ % 4) * 128:(n_ % 4 + 1) * 128] = a[8 * n_:8 * n_ + 8]

    def proj_qv(i, g, xn):
        for b in range(TM // 128):
            r0 = i * TM + b * 128
            qv = lax.dot_general(
                pltpu.bitcast(wqvt_s[g * 128:(g + 1) * 128, :], bf16),
                xn[b * 128:(b + 1) * 128], NT, preferred_element_type=f32)
            for j in range(8):
                h = g * 8 + j
                qh = (qv[32 * j:32 * j + 16] * QSCALE).astype(bf16)
                qt_s[h * 8:h * 8 + 8, r0:r0 + 128] = pltpu.bitcast(qh, u32)
                qb_s[h * 16 + r0 // 128] = jnp.broadcast_to(
                    qh.astype(f32)[:, None, :], (DH, 8, 128))
                v = qv[32 * j + 16:32 * j + 32]
                vt_s[h * 8:h * 8 + 8, r0:r0 + 128] = _to_u32(v)
                va = jnp.maximum(jnp.abs(v[0:8]), jnp.abs(v[8:16]))
                vmax[0] = va if vmax[0] is None else jnp.maximum(vmax[0], va)

    def ln1(i):
        return _ln(x_ref[i * TM:(i + 1) * TM, :].astype(f32)).astype(bf16)

    cp_x[0].wait()
    cp_w[2].start()
    cp_w[3].start()
    xn0 = ln1(0)
    cp_w[0].wait()
    cp_w[1].wait()
    cp_w[4].start()
    cp_x[1].start()
    for g in range(2):
        transpose_w(g)
        proj_qv(0, g, xn0)
    cp_w[2].wait()
    cp_w[3].wait()
    cp_x[2].start()
    for g in range(2, 4):
        transpose_w(g)
        proj_qv(0, g, xn0)
    cp_w[4].wait()
    cp_x[1].wait()
    for cp in (cp_o, cp_r, cp_g, cp_u, cp_d):
        cp.start(priority=1)
    xn1 = ln1(1)
    proj_k(0, 0, xn0)
    for g in range(3):
        proj_k(0, g + 1, xn0)
        proj_qv(1, g, xn1)
    cp_x[2].wait()
    proj_qv(1, 3, xn1)
    for i in range(2, NTILE):
        xn = ln1(i)
        for g in range(4):
            if i == 2:
                proj_k(1, g, xn1)
            proj_k(i, g, xn)
            proj_qv(i, g, xn)
    l_s[0:8, 0:128] = vmax[0] * (L_MAX / V_MAX)

    def ld(row, n, z8):
        return pltpu.bitcast(mem[pl.ds(pl.multiple_of(row + z8, 8), n), :], f32)

    def st(row, v):
        mem[row:row + v.shape[0], :] = pltpu.bitcast(v, u32)

    def make_kb(h, par, c, ds_, zi, anc=None, never=None):
        lane = lax.broadcasted_iota(i32, (RV, 128), 1)
        kk = pltpu.bitcast(
            k_s[pl.ds(pl.multiple_of((h + zi) * NC * 16 + c * 16 + 8, 8), 8), 384:512],
            bf16).astype(f32)
        if anc is not None:
            kk = jnp.where(never, anc, kk)
        for d in ds_:
            col = jnp.sum(jnp.where(lane == d, kk, 0.0), axis=1, keepdims=True)
            kb_s[par][0, c, d] = jnp.broadcast_to(col, (RV, 128))

    def vpu_scores(c, kpar, t, zi, never):
        res = []
        qbase = qb_s.at[pl.ds(t[0] * 16 + zi + t[1] * 4, 4)]
        for j in range(4):
            zz = z_s[NZ + j] + zi
            acc = None
            for d in range(DH):
                qb = jnp.tile(qbase[j, d], (2, 1))
                kb = kb_s[kpar][zz, c, d]
                if acc is None:
                    acc = kb * qb
                    if res:
                        acc = jnp.where(never, res[-1], acc)
                else:
                    acc = acc + kb * qb
            res.append(acc)
        return jnp.concatenate(res, axis=1)

    def fin(t, par, l, zi):
        h, qi = t
        lt = jnp.sum(l, axis=0, keepdims=True)
        l_s[pl.ds(8 + h, 1), qi * TQ:(qi + 1) * TQ] = lt
        acc = ld(AB + par * 16, 16, zi * 8)
        ot_s[pl.ds(pl.multiple_of(h * 8, 8), 8), qi * TQ:(qi + 1) * TQ] = _to_u32(
            acc * pl.reciprocal(lt, approx=True))

    def k_blocks(h, c, z8, nb):
        row = h * NC * 16 + z8 + c * 16
        return jnp.concatenate(
            [k_s[pl.ds(pl.multiple_of(row + (i // 4) * 8, 8), 8),
                 (i % 4) * 128:(i % 4 + 1) * 128] for i in range(nb)], axis=0)

    for c in range(NC):
        make_kb(0, 0, c, range(DH), 0)

    def run(it, l, tail):
        never = jnp.full((16, 128), z_s[NZ + 7], i32) != 0
        tp = (jnp.maximum(it * HB - 1, 0), NQ - 1)
        pend = [(NC - PL + i, -1, tp, (NZ - PL + i) % RING, NB if i else 8)
                for i in range(PL)]
        L = {-1: l}
        accq = []

        def flush(keep, zi):
            while len(accq) > keep:
                a, cc, uu, tt = accq.pop(0)
                r = AB + (uu % 2) * 16
                st(r, a if cc == 0 else ld(r, 16, zi * 8) + a)
                if cc == NC - 1:
                    fin(tt, uu % 2, L[uu], zi)

        def step(qk, prev, zi):
            cc, uu, tt, sl, nb = pend.pop(0)
            z8 = zi * 8
            done = [0]

            def stores(want):
                if prev is None:
                    return
                while done[0] < min(want, prev[0].shape[0] // 16):
                    i = done[0]
                    st(prev[1] * KC + 16 * i, prev[0][16 * i:16 * i + 16])
                    done[0] += 1

            P = [None] * 8
            l = L[uu]
            for k, pos in enumerate(range(7, -1, -1)):
                stores(max(k + 1 - OFF, 0))
                if k == AK:
                    flush(1, zi)
                if pos == VB and nb == NB:
                    sb = vpu_scores(cc, (uu // NQ) % 2, tt, zi, never)
                else:
                    sb = ld(sl * KC + 16 * SLOT.index(pos), 16, z8)
                p = jnp.exp2(sb)
                P[pos] = p
                for x in (p[0:8], p[8:16]):
                    l = x if l is None else l + x
            stores(8)
            L[uu] = l
            s = None
            if qk is not None:
                c, t, nbq = qk
                h, qi = t
                kk = pltpu.bitcast(k_blocks(h, c, z8, nbq), bf16)
                qh = qt_s[pl.ds(pl.multiple_of(h * 8 + z8, 8), 8), qi * TQ:(qi + 1) * TQ]
                w = pltpu.bitcast(
                    jnp.concatenate([qh, jnp.zeros((56, TQ), u32)], axis=0), bf16)
                s = jnp.dot(kk, w, preferred_element_type=f32)
            hoff = pl.multiple_of(tt[0] * 8, 8)
            vt = pltpu.bitcast(vt_s[pl.ds(hoff, 8), cc * KC:(cc + 1) * KC], bf16)
            a = jnp.dot(vt, jnp.concatenate(P, axis=0).astype(bf16),
                        preferred_element_type=f32)
            accq.append((a, cc, uu, tt))
            return s

        if tail:
            while pend:
                step(None, None, z_s[len(pend)])
            flush(0, z_s[0])
            return None
        n = 0
        prev = None
        for u in range(NSUB):
            t = (it * HB + u // NQ, u % NQ)
            L[u] = None
            for c in range(NC):
                zi = z_s[n]
                nb = 8 if n == NZ - PL else NB
                pend.append((c, u, t, n % RING, nb))
                s = step((c, t, nb), prev, zi)
                anc = prev[0][0:16, 0:128] if prev is not None else None
                prev = (s, n % RING)
                hh = u // NQ
                for gc, gd in GSCHED.get((u % NQ) * NC + c, {}).items():
                    make_kb(jnp.minimum(it * HB + hh + 1, H - 1), (hh + 1) % 2, gc, gd,
                            zi, anc, never)
                n += 1
        st(prev[1] * KC, prev[0])
        flush(0, z_s[0])
        return L[NSUB - 1]

    l_end = lax.fori_loop(0, H // HB, lambda it, l: run(it, l, False),
                          jnp.ones((8, TQ), f32))
    for cp in (cp_o, cp_r, cp_g, cp_u, cp_d):
        cp.wait()
    run(H // HB, l_end, True)

    wr = jnp.broadcast_to(wr_ref[...].astype(f32).reshape(1, D), (16, D)).astype(bf16)
    tiles = [slice(i * TM, (i + 1) * TM) for i in range(NTILE)]
    cp_out = [pltpu.make_async_copy(o_ref.at[tiles[i]], o_hbm.at[tiles[i]], osem.at[i])
              for i in range(NTILE)]

    def project(rows):
        ot = pltpu.bitcast(ot_s[:, rows], bf16)
        return lax.dot_general(ot, wo_ref[...], TN, preferred_element_type=f32)

    def finish(rows, attn_out, cp):
        h = x_ref[rows, :].astype(f32) + attn_out
        xn2f = _ln(h)
        xn2 = xn2f.astype(bf16)
        xn2_s[rows, :] = xn2
        o_ref[rows, :] = (h + xn2f).astype(bf16)
        if cp is not None:
            cp.start()
        r = lax.dot_general(wr, xn2, NT, preferred_element_type=f32)
        r_s[:, rows] = r[0:8]

    def route(before_update):
        bits = pltpu.bitcast(r_s[...].astype(bf16).astype(f32), i32) >> 16
        srt = bits ^ ((bits >> 15) & 0x7FFF)
        idx = lax.broadcasted_iota(i32, (8, S), 1)
        key = srt * S + (S - 1 - idx)
        kv1 = jnp.max(key, axis=1, keepdims=True)
        kv2 = jnp.max(jnp.where(key == kv1, jnp.iinfo(jnp.int32).min, key),
                      axis=1, keepdims=True)
        key1 = jnp.max(kv1)
        key2 = jnp.max(kv2)
        i1 = S - 1 - (key1 & (S - 1))
        i2 = S - 1 - (key2 & (S - 1))

        row16 = lax.broadcasted_iota(i32, (16, D), 0)
        b1 = pl.multiple_of(jnp.clip((i1 // 16) * 16, 0, S - 16), 16)
        b2 = pl.multiple_of(jnp.clip((i2 // 16) * 16, 0, S - 16), 16)
        blk1 = xn2_s[pl.ds(b1, 16), :].astype(f32)
        blk2 = xn2_s[pl.ds(b2, 16), :].astype(f32)
        x1 = jnp.sum(jnp.where(row16 == i1 % 16, blk1, 0.0), axis=0, keepdims=True)
        x2 = jnp.sum(jnp.where(row16 == i2 % 16, blk2, 0.0), axis=0, keepdims=True)
        xs = jnp.where(row16 == 0, x1, jnp.where(row16 == 1, x2, 0.0)).astype(bf16)

        g = jnp.dot(xs, wg_s[...], preferred_element_type=f32)
        g = g * jax.nn.sigmoid(g)
        uu = jnp.dot(xs, wu_s[...], preferred_element_type=f32)
        y = jnp.dot((g * uu).astype(bf16), wd_s[...], preferred_element_type=f32)
        ks = jnp.where(row16 == 0, key1, key2) >> 11
        rsel = pltpu.bitcast((ks ^ ((ks >> 15) & 0x7FFF)) << 16, f32)
        y = y * jax.nn.sigmoid(rsel)

        before_update()
        ob = o_ref[pl.ds(b1, 16), :].astype(f32)
        o_ref[pl.ds(b1, 16), :] = jnp.where(row16 == i1 % 16, ob + y[0:1], ob).astype(bf16)
        ob = o_ref[pl.ds(b2, 16), :].astype(f32)
        o_ref[pl.ds(b2, 16), :] = jnp.where(row16 == i2 % 16, ob + y[1:2], ob).astype(bf16)
        return b1, b2

    nxt = project(tiles[0])
    for i in range(NTILE):
        cur = nxt
        if i + 1 < NTILE:
            nxt = project(tiles[i + 1])
        finish(tiles[i], cur, cp_out[i])

    parts = [l_s[8 * a:8 * a + 8, 128 * b:128 * b + 128]
             for a in range(1, 1 + H // 8) for b in range(S // 128)]
    lmax = functools.reduce(jnp.maximum, parts + [l_s[0:8, 0:128]])
    lmin = functools.reduce(jnp.minimum, parts)
    ok = jnp.max(jnp.where(lmin >= L_MIN, lmax, jnp.inf)) <= L_MAX

    def wait_out():
        for i in range(NTILE):
            cp_out[i].wait()

    b1, b2 = route(wait_out)
    fix1 = pltpu.make_async_copy(o_ref.at[pl.ds(b1, 16)], o_hbm.at[pl.ds(b1, 16)], osem.at[0])
    fix2 = pltpu.make_async_copy(o_ref.at[pl.ds(b2, 16)], o_hbm.at[pl.ds(b2, 16)], osem.at[1])
    fix1.start()

    @pl.when(b1 != b2)
    def _():
        fix2.start()
        fix2.wait()

    fix1.wait()

    @pl.when(jnp.logical_not(ok))
    def _():
        def exact(t, carry):
            h = t // 16
            q0 = pl.multiple_of((t % 16) * 128, 128)
            rows = []
            for c in range(NC):
                km = k_blocks(h, c, 0, 8)
                for p in range(8):
                    n_ = SLOT.index(p)
                    rows.append(km[8 * n_:8 * n_ + 8])
            kk = pltpu.bitcast(jnp.concatenate(rows, axis=0), bf16)
            qh = qt_s[pl.ds(pl.multiple_of(h * 8, 8), 8), pl.ds(q0, 128)]
            w = pltpu.bitcast(
                jnp.concatenate([qh, jnp.zeros((56, 128), u32)], axis=0), bf16)
            s = jnp.dot(kk, w, preferred_element_type=f32)
            p = jnp.exp2(s - jnp.max(s, axis=0, keepdims=True))
            p = p * pl.reciprocal(jnp.sum(p, axis=0, keepdims=True), approx=False)
            vt = pltpu.bitcast(vt_s[pl.ds(pl.multiple_of(h * 8, 8), 8), :], bf16)
            ot_s[pl.ds(pl.multiple_of(h * 8, 8), 8), pl.ds(q0, 128)] = _to_u32(
                jnp.dot(vt, p.astype(bf16), preferred_element_type=f32))
            return carry

        lax.fori_loop(0, H * 16, exact, 0)

        def redo(i, carry):
            rows = pl.ds(pl.multiple_of(i * 128, 128), 128)
            finish(rows, project(rows), None)
            return carry

        lax.fori_loop(0, S // 128, redo, 0)
        route(lambda: None)
        cp_all = pltpu.make_async_copy(o_ref, o_hbm, osem.at[0])
        cp_all.start()
        cp_all.wait()


@jax.jit
def pallas_sequential_preLN__mha_block__moe_arch_mod__prompt_kernel(
    A_x: jax.Array,
    A_wqkv: jax.Array,
    A_wo: jax.Array,
    B_x: jax.Array,
    B_w_r: jax.Array,
    B_w_gate: jax.Array,
    B_w_up: jax.Array,
    B_w_down: jax.Array,
):
    del B_x
    hbm = pl.BlockSpec(memory_space=pl.ANY)
    out = pl.pallas_call(
        _kernel,
        out_shape=jax.ShapeDtypeStruct((S, D), bf16),
        in_specs=[hbm] * 7,
        out_specs=hbm,
        scratch_shapes=[
            pltpu.VMEM((S, D), bf16),
            pltpu.VMEM((D, 3 * D), bf16),
            pltpu.VMEM((D, D), bf16),
            pltpu.VMEM((D,), bf16),
            pltpu.VMEM((D, F), bf16),
            pltpu.VMEM((D, F), bf16),
            pltpu.VMEM((F, D), bf16),
            pltpu.VMEM((S, D), bf16),
            pltpu.SemaphoreType.DMA((3,)),
            pltpu.SemaphoreType.DMA((13,)),
            pltpu.SemaphoreType.DMA((NTILE,)),
            pltpu.VMEM((D, D), u32),
            pltpu.VMEM((H * NC * 16, D), u32),
            pltpu.VMEM((MR, D), u32),
            pltpu.VMEM((D // 2, S), u32),
            pltpu.VMEM((D // 2, S), u32),
            pltpu.VMEM((D // 2, S), u32),
            pltpu.VMEM((H * 16, DH, 8, 128), f32),
            pltpu.VMEM((1, NC, DH, RV, 128), f32),
            pltpu.VMEM((1, NC, DH, RV, 128), f32),
            pltpu.SMEM((NZ + 8,), i32),
            pltpu.VMEM((8 + H, S), f32),
            pltpu.VMEM((S, D), bf16),
            pltpu.VMEM((8, S), f32),
        ],
        compiler_params=pltpu.CompilerParams(vmem_limit_bytes=112 * 1024 * 1024),
        name="preln_mha_mod",
    )(A_x.reshape(S, D), A_wqkv, A_wo, B_w_r, B_w_gate, B_w_up, B_w_down)
    return out.reshape(1, S, D)
```
